```python
import os as _os
_os.environ.setdefault("JAX_PLATFORMS", "cpu")
import jax
import jax.numpy as jnp

def _softmax(x, axis=-1):
    return jax.nn.softmax(x, axis=axis)
def _gelu(x):
    return jax.nn.gelu(x, approximate=True)
def _silu(x):
    return jax.nn.silu(x)
def _sigmoid(x):
    return jax.nn.sigmoid(x)
def _layernorm(x, axis=-1, eps=1e-5):
    m = jnp.mean(x, axis=axis, keepdims=True)
    v = jnp.var(x, axis=axis, keepdims=True)
    return (x - m) / jnp.sqrt(v + eps)
def _scatter_add(tgt, idx, src, axis=0):
    return tgt.at[idx].add(src)
def _segment_sum(src, seg, n):
    return jax.ops.segment_sum(src, seg, n)
class _Rng:
    def __init__(self, key):
        self._k = key
    def _next(self):
        self._k, sub = jax.random.split(self._k)
        return sub
    def normal(self, shape):
        return jax.random.normal(self._next(), shape, dtype=jnp.bfloat16)
    def randint(self, lo, hi, shape):
        return jax.random.randint(self._next(), shape, lo, hi, dtype=jnp.int32)
    def uniform(self, shape, lo=0.0, hi=1.0):
        return jax.random.uniform(self._next(), shape, jnp.bfloat16, lo, hi)
    def permutation(self, n):
        return jax.random.permutation(self._next(), n)


kernel_name = 'concat_heads__sliding_local_dilated__compressed_kv_cla__prompt'

def setup_inputs():
    _rng = _Rng(jax.random.key(int.from_bytes(__import__("os").urandom(4), "little")))
    _w = (lambda a: (lambda t: t.astype(jnp.bfloat16) if jnp.issubdtype(t.dtype, jnp.floating) else t)(jnp.asarray(a)))
    def _A_setup():
        B, S, D = 1, 2048, 640
        return {
            "x": _w((lambda *s: _rng.normal(s) * 0.2)(B, S, D)),
            "wqkv": _w((lambda *s: _rng.normal(s) * 0.2)(D, 3 * D)),
            "wo": _w((lambda *s: _rng.normal(s) * 0.05)(D, D)),
        }
    _A_in = _A_setup()

    def _B_setup():
        B, H, Sq, Sk, D, M = 1, 32, 2048, 2048, 128, 640
        Dc = 4 * D
        return {
            "x": _w((lambda *s: _rng.normal(s) * 0.8)(B, Sq, M)),
            "c_kv": _w((lambda *s: _rng.normal(s) * 0.8)(B, Sk, Dc)),
            "w_q": _w((lambda *s: _rng.normal(s) * 1.6)(M, H, D) * (M ** -0.5)),
            "w_uk": _w((lambda *s: _rng.normal(s) * 1.6)(Dc, H, D) * (Dc ** -0.5)),
            "w_uv": _w((lambda *s: _rng.normal(s) * 0.8)(Dc, H, D) * (Dc ** -0.5)),
            "w_o": _w((lambda *s: _rng.normal(s) * 0.8)(H, D, M) * ((H * D) ** -0.5)),
        }
    _B_in = _B_setup()

    return {
        "A_x": _A_in["x"],
        "A_wqkv": _A_in["wqkv"],
        "A_wo": _A_in["wo"],
        "B_x": _B_in["x"],
        "B_c_kv": _B_in["c_kv"],
        "B_w_q": _B_in["w_q"],
        "B_w_uk": _B_in["w_uk"],
        "B_w_uv": _B_in["w_uv"],
        "B_w_o": _B_in["w_o"],
    }

def reference(A_x, A_wqkv, A_wo, B_x, B_c_kv, B_w_q, B_w_uk, B_w_uv, B_w_o):
    def _A_ref(x, wqkv, wo):
        B, S, D = x.shape
        H = 32; Dh = D // H
        W, dil = 8, 2
        qkv = (lambda x, *d: x.transpose(*d))((x @ wqkv).reshape(B, S, 3, H, Dh), 2, 0, 3, 1, 4)
        q, k, v = qkv[0], qkv[1], qkv[2]
        scale = Dh ** -0.5
        pos = jnp.arange(S)
        off = jnp.arange(W) * dil
        idx = pos[:, None] - off[None, :]
        mask = idx >= 0
        idx_c = jnp.where(mask, idx, 0).reshape(-1)
        kg = k[:, :, idx_c, :].reshape(B, H, S, W, Dh)
        vg = v[:, :, idx_c, :].reshape(B, H, S, W, Dh)
        logits = jnp.einsum("bhsd,bhswd->bhsw", q, kg) * scale
        logits = jnp.where(mask[None, None, :, :], logits, -1e9)
        attn = _softmax(logits, axis=-1)
        o = jnp.einsum("bhsw,bhswd->bhsd", attn, vg)
        return (lambda x, *d: x.transpose(*d))(o, 0, 2, 1, 3).reshape(B, S, D) @ wo

    def _B_ref(x, c_kv, w_q, w_uk, w_uv, w_o):
        B, Sq, M = x.shape[0], x.shape[1], x.shape[2]
        Sk = c_kv.shape[1]
        H, D = w_q.shape[1], w_q.shape[2]
        q = jnp.einsum("bqm,mhd->bhqd", x, w_q)
        k = jnp.einsum("bkc,chd->bhkd", c_kv, w_uk)
        v = jnp.einsum("bkc,chd->bhkd", c_kv, w_uv)
        scores = jnp.einsum("bhqd,bhkd->bhqk", q, k) * (D ** -0.5)
        off = Sk - Sq
        qi = jnp.arange(Sq)[:, None]
        kj = jnp.arange(Sk)[None, :]
        cmask = kj <= (qi + off)
        scores = jnp.where(cmask[None, None], scores, -1e9)
        p = _softmax(scores, axis=-1)
        ctx = jnp.einsum("bhqk,bhkd->bhqd", p, v)
        return jnp.einsum("bhqd,hdm->bqm", ctx, w_o)

    a = _A_ref(A_x, A_wqkv, A_wo)
    b = _B_ref(B_x, B_c_kv, B_w_q, B_w_uk, B_w_uv, B_w_o)
    return jnp.concatenate([a, b], axis=-1)
```

```python
import functools
import math

import jax
import jax.numpy as jnp
from jax import lax
import jax.experimental.pallas as pl
import jax.experimental.pallas.tpu as pltpu

f32 = jnp.float32
bf16 = jnp.bfloat16
u32 = jnp.uint32

S = 2048
M = 640
HA = 32
DA = 20
WIN = 8
DIL = 2
PAD = 16
RA = 512
NA = S // RA
G = M // 128
H = 32
D = 128
DC = 512
BQ = 512
PC = 256
KC = 256
PVK = 4
RS = S // H

LOG2E = math.log2(math.e)
QSCALE_A = (DA ** -0.5) * LOG2E
QSCALE_B = (D ** -0.5) * LOG2E
NEG = -1e9 * LOG2E
NT = (((1,), (1,)), ((), ()))
HI_MASK = 0xFFFF0000
SCOPES = False
NV = 0
APOS = 10
VAR = 3
HPS = 2


class _NoScope:
    def __enter__(self):
        return self

    def __exit__(self, *a):
        return False


def _scope(name):
    return jax.named_scope(name) if SCOPES else _NoScope()


def _tree(parts, op):
    parts = list(parts)
    while len(parts) > 1:
        nxt = [op(parts[a], parts[a + 1]) for a in range(0, len(parts) - 1, 2)]
        if len(parts) % 2:
            nxt.append(parts[-1])
        parts = nxt
    return parts[0]


def _fold8(x, op):
    n = x.shape[0] // 8
    return _tree([x[j * 8:(j + 1) * 8] for j in range(n)], op)


def _interleave(heavy, light):
    th = sum(c for c, _ in heavy)
    tl = sum(c for c, _ in light)
    out = []
    ih = il = 0
    dh = dl = 0
    while ih < len(heavy) or il < len(light):
        fh = dh / th if th else 1.0
        fl = dl / tl if tl else 1.0
        if il < len(light) and (ih >= len(heavy) or fl <= fh):
            out.append(light[il]); dl += light[il][0]; il += 1
        else:
            out.append(heavy[ih]); dh += heavy[ih][0]; ih += 1
    return out


def _kernel(ax_hbm, aw_hbm, awo_hbm, bx_hbm, bc_hbm, wq_hbm, wk_hbm, wv_hbm, wo_hbm,
            out_hbm,
            ax_s, aw_s, awo_s, t_s, wt_s, wop_s, qa_s, ka_s, va_s, oa_s,
            bx_s, bc_s, wq32, wk32, wv32, wo_s, wqh, wkh, wvth,
            q_s, k_s, vt_s, s0, s1, s2, s3, s4, s5, s6, s7, acc_ref, ob_s,
            z_s, sem_in, sem_w, sem_out):
    step = pl.program_id(0)

    def cp_aw(sec):
        return pltpu.make_async_copy(aw_hbm.at[:, pl.ds(sec * M, M)], aw_s.at[:, pl.ds(sec * M, M)], sem_in.at[sec])

    def cp_ax(c):
        return pltpu.make_async_copy(ax_hbm.at[pl.ds(c * RA, RA)], ax_s.at[pl.ds(c * RA, RA)], sem_in.at[9 + c])
    cp_awo = pltpu.make_async_copy(awo_hbm, awo_s, sem_in.at[5])
    cp_b = [
        pltpu.make_async_copy(bx_hbm, bx_s, sem_in.at[6]),
        pltpu.make_async_copy(bc_hbm, bc_s, sem_in.at[7]),
        pltpu.make_async_copy(wo_hbm, wo_s, sem_in.at[8]),
    ]

    def cp_w(hn, slot):
        j = hn >> 1 if isinstance(hn, int) else lax.shift_right_logical(hn, 1)
        return [
            pltpu.make_async_copy(src.bitcast(u32).at[:, j, :], dst.at[slot], sem_w.at[slot, i])
            for i, (src, dst) in enumerate(((wq_hbm, wq32), (wk_hbm, wk32), (wv_hbm, wv32)))
        ]

    def cp_oa(r0):
        return pltpu.make_async_copy(oa_s.at[pl.ds(r0, RS * HPS)], out_hbm.at[pl.ds(r0, RS * HPS), pl.ds(0, M)],
                                     sem_out.at[0])

    def cp_ob(c):
        return pltpu.make_async_copy(ob_s.at[pl.ds(c * PC, PC)], out_hbm.at[pl.ds(c * PC, PC), pl.ds(M, M)],
                                     sem_out.at[1 + c])

    def unpack(w32, hn, slot):
        w = w32[slot]
        if isinstance(hn, int):
            w = (w & jnp.uint32(HI_MASK)) if hn & 1 else (w << 16)
        else:
            w = (w << ((1 - (hn & 1)) * 16).astype(u32)) & jnp.uint32(HI_MASK)
        return pltpu.bitcast(w, f32)

    def ext_q(hn, slot):
        wqh[...] = unpack(wq32, hn, slot).astype(bf16)

    def ext_k(hn, slot):
        wkh[...] = unpack(wk32, hn, slot).astype(bf16)

    def ext_v(hn, slot):
        wvth[...] = unpack(wv32, hn, slot).T.astype(bf16)

    def prep_w(sec):
        for cb in range(G):
            c0 = sec * M + cb * 128
            for g in range(G):
                t_s[g, c0:c0 + 128, :] = aw_s[g * 128:(g + 1) * 128, c0:c0 + 128].astype(f32).T
        for d in range(DA):
            for g in range(G):
                wt_s[sec * M + d * HA:sec * M + (d + 1) * HA, g * 128:(g + 1) * 128] = (
                    t_s[g, pl.ds(sec * M + d, HA, stride=DA), :].astype(bf16))

    def prep_wo():
        for g in range(G):
            t_s[g, 0:M, :] = awo_s[:, g * 128:(g + 1) * 128].astype(f32)
        for d in range(DA):
            for g in range(G):
                wop_s[d * HA:(d + 1) * HA, g * 128:(g + 1) * 128] = (
                    t_s[g, pl.ds(d, HA, stride=DA), :].astype(bf16))

    def a_proj(rbase, secs=(0, 1, 2)):
        for sec in secs:
            for sub in range(RA // PC):
                r0 = rbase + sub * PC
                r = lax.dot_general(ax_s[pl.ds(r0, PC), :], wt_s[sec * M:(sec + 1) * M, :], NT,
                                    preferred_element_type=f32)
                for g in range(G):
                    t = r[:, g * 128:(g + 1) * 128]
                    if sec == 0:
                        qa_s[g, pl.ds(r0, PC), :] = t * QSCALE_A
                    elif sec == 1:
                        ka_s[g, pl.ds(r0 + PAD, PC), :] = t
                    else:
                        va_s[g, pl.ds(r0 + PAD, PC), :] = t

    def a_attn(rr):
        q = [qa_s[g, pl.ds(rr, RS), :] for g in range(G)]
        rowid = rr + lax.broadcasted_iota(jnp.int32, (PAD, 128), 0)
        lg = []
        for w in range(WIN):
            acc = _tree([q[g] * ka_s[g, pl.ds(rr + (PAD - DIL * w), RS), :] for g in range(G)], jnp.add)
            acc = acc + pltpu.roll(acc, 64, 1)
            acc = acc + pltpu.roll(acc, 32, 1)
            if w > 0:
                top = jnp.where(rowid >= DIL * w, acc[:PAD], NEG)
                acc = jnp.concatenate([top, acc[PAD:]], axis=0)
            lg.append(acc)
        m = _tree(lg, jnp.maximum)
        e = [jnp.exp2(x - m) for x in lg]
        inv = pl.reciprocal(_tree(e, jnp.add), approx=False)
        og = []
        for g in range(G):
            acc = _tree([e[w] * va_s[g, pl.ds(rr + (PAD - DIL * w), RS), :] for w in range(WIN)], jnp.add)
            og.append(acc * inv)
        return jnp.concatenate(og, axis=1).astype(bf16)

    @pl.when(step == 0)
    def _prologue():
      with _scope("prologue"):
        cp_aw(0).start()
        cp_ax(0).start()
        cp_aw(1).start()
        cp_ax(1).start()
        cp_aw(2).start()
        z_s[0] = 0
        z_s[1] = 0
        zero = jnp.zeros((PAD, 128), f32)
        for g in range(G):
            ka_s[g, 0:PAD, :] = zero
            va_s[g, 0:PAD, :] = zero
        acc_ref[...] = jnp.zeros_like(acc_ref)
        cp_aw(0).wait()
        for c in range(2, NA):
            cp_ax(c).start()
        cp_awo.start()
        cp_ax(0).wait()
        prep_w(0)
        a_proj(0, (0,))
        cp_aw(1).wait()
        cp_ax(1).wait()
        for cp in cp_w(0, 0):
            cp.start()
        for cp in cp_b:
            cp.start()
        a_proj(RA, (0,))
        prep_w(1)
        a_proj(0, (1,))
        cp_aw(2).wait()
        cp_ax(2).wait()
        cp_awo.wait()
        cp_ax(3).wait()
        a_proj(2 * RA, (0,))
        prep_wo()
        a_proj(3 * RA, (0,))
        prep_w(2)
        a_proj(0, (2,))

        def body(c, carry):
            a_proj(pl.multiple_of(c * RA, RA), (1, 2))
            return carry
        with _scope("a_loop"):
            lax.fori_loop(1, NA, body, 0)
        for cp in cp_b:
            cp.wait()

    NSTEP = H // HPS
    RST = RS * HPS
    slot = step & 1
    h0 = step * HPS
    for cp in cp_w(h0, slot):
        cp.wait()

    @pl.when(step >= 2)
    def _():
        cp_oa(pl.multiple_of((step - 2) * RST, RST)).wait()

    @pl.when(step + 1 < NSTEP)
    def _():
        for cp in cp_w(h0 + HPS, 1 - slot):
            cp.start()

    @pl.when(step >= 1)
    def _():
        cp_oa(pl.multiple_of((step - 1) * RST, RST)).start()

    def head(hh):
        h = h0 + hh
        par = hh if HPS % 2 == 0 else h
        last = hh == HPS - 1
        zs = z_s[0]
        zl = z_s[1]
        sb = [s0, s1, s2, s3] if hh % 2 == 0 else [s4, s5, s6, s7]
        row = lax.broadcasted_iota(jnp.int32, (128, 128), 0)
        col = lax.broadcasted_iota(jnp.int32, (128, 128), 1)
        tri = row <= col
        ra = pl.multiple_of(h * RS, RS)

        pm = {}
        mx = {}
        ot = {}
        ls = {}
        ob = {}
        oa = {}

        def Pq(a):
            def f():
                q_s[a:a + PC, :] = (jnp.dot(bx_s[a:a + PC, :], wqh[...], preferred_element_type=f32) * QSCALE_B).astype(bf16)
            return (PC // 16 * 5, f)

        def Pk(a):
            def f():
                k_s[a:a + PC, :] = jnp.dot(bc_s[a:a + PC, :], wkh[...], preferred_element_type=f32).astype(bf16)
            return (PC // 16 * 4, f)

        def Pv(a):
            def f():
                vt_s[:, a:a + PC] = lax.dot_general(wvth[...], bc_s[a:a + PC, :], NT, preferred_element_type=f32).astype(bf16)
            return (PC // 16 * 4, f)

        def QKq(i, k0, k1, t0):
            lo = i * BQ

            def f():
                r = lax.dot_general(k_s[k0:k1, :], q_s[lo + t0 * 128:lo + BQ, :], NT, preferred_element_type=f32)
                for t in range(t0, 4):
                    c = i * 4 + t
                    for j in range(k0 // 128, k1 // 128):
                        tile = r[j * 128 - k0:(j + 1) * 128 - k0, (t - t0) * 128:(t - t0 + 1) * 128]
                        if j == c:
                            tile = jnp.where(tri, tile, NEG)
                        sb[i][zs + t, j * 128:(j + 1) * 128, :] = tile
                        pm.setdefault(c, []).append(_fold8(tile, jnp.maximum))
            return ((k1 - k0) // 16 * (4 - t0), f)

        def QK(i):
            lo = i * BQ
            qs = []
            k0 = 0
            while k0 < lo + 128:
                k1 = min(k0 + KC, lo + 128)
                qs.append(QKq(i, k0, k1, 0))
                k0 = k1
            for u in range(1, 4):
                qs.append(QKq(i, lo + u * 128, lo + (u + 1) * 128, u))
            return qs

        def PVq(c, j0, j1):
            def f():
                if c not in mx:
                    mx[c] = jnp.max(_tree(pm.pop(c), jnp.maximum), axis=0, keepdims=True)
                p = jnp.exp2(sb[c // 4][zl + c % 4, j0 * 128:j1 * 128, :] - mx[c])
                lsum = _fold8(p, jnp.add)
                ls[c] = lsum if c not in ls else ls[c] + lsum
                o = jnp.dot(vt_s[:, j0 * 128:j1 * 128], p.astype(bf16), preferred_element_type=f32)
                ot[c] = o if c not in ot else ot[c] + o
                if j1 == c + 1:
                    l = jnp.sum(ls.pop(c), axis=0, keepdims=True)
                    ob[c] = (ot.pop(c) * pl.reciprocal(l, approx=False)).T
            return ((j1 - j0) * 8, f)

        def PV(i):
            qs = []
            for t in range(4):
                c = i * 4 + t
                for j0 in range(0, c + 1, PVK):
                    qs.append(PVq(c, j0, min(j0 + PVK, c + 1)))
            return qs

        def OPq(a):
            def f():
                cs = range(a // 128, (a + PC) // 128)
                o = jnp.concatenate([ob.pop(c) for c in cs], axis=0).astype(bf16)
                new = acc_ref[a:a + PC, :] + jnp.dot(o, wo_s[h], preferred_element_type=f32)
                acc_ref[a:a + PC, :] = new
                if last:
                    ob_s[a:a + PC, :] = new.astype(bf16)

                    @pl.when(step == NSTEP - 1)
                    def _():
                        cp_ob(a // PC).start()
            return (PC // 16 * 5, f)

        def do(fn, *args):
            return (0, lambda: fn(*args))

        def Aattn():
            oa[0] = a_attn(ra)

        def Aout():
            oa_s[pl.ds(ra, RS), :] = jnp.dot(oa.pop(0), wop_s[...], preferred_element_type=f32).astype(bf16)

        def rows(i):
            return range(i * BQ, (i + 1) * BQ, PC)

        seq = [do(ext_q, par, slot), do(ext_k, par, slot), do(ext_v, par, slot), do(Aattn)]
        qk3 = QK(3)
        pvs = [Pv(a) for a in range(0, S, PC)]
        pks = [Pk(a) for a in range(0, S, PC)]
        pre = [Pq(a) for a in rows(3)] + pks + pvs[:NV] + qk3 + [Pq(a) for a in rows(2)] + pvs[NV:]
        seq += pre[:APOS] + [do(Aout)] + pre[APOS:]
        if VAR == 0:
            seq += _interleave(PV(3), QK(2) + [Pq(a) for a in rows(1)])
            seq += _interleave(PV(2), QK(1) + [Pq(a) for a in rows(0)] + [OPq(a) for a in rows(3)])
            seq += _interleave(PV(1), QK(0) + [OPq(a) for a in rows(2)])
            seq += PV(0) + [OPq(a) for a in rows(1)] + [OPq(a) for a in rows(0)]
        elif VAR == 1:
            seq += _interleave(PV(3), QK(2) + [Pq(a) for a in rows(1)] + [Pq(a) for a in rows(0)])
            seq += _interleave(PV(2), QK(1) + QK(0) + [OPq(a) for a in rows(3)])
            seq += _interleave(PV(1) + PV(0), [OPq(a) for a in rows(2)])
            seq += [OPq(a) for a in rows(1)] + [OPq(a) for a in rows(0)]
        elif VAR == 2:
            seq += _interleave(PV(3), QK(2) + [Pq(a) for a in rows(1)])
            seq += _interleave(PV(2), QK(1) + [OPq(a) for a in rows(3)] + [Pq(a) for a in rows(0)])
            seq += _interleave(PV(1), [OPq(a) for a in rows(2)][:1] + QK(0) + [OPq(a) for a in rows(2)][1:])
            seq += _interleave(PV(0), [OPq(a) for a in rows(1)]) + [OPq(a) for a in rows(0)]
        elif VAR == 3:
            seq += _interleave(PV(3), [Pq(a) for a in rows(1)] + QK(2))
            seq += _interleave(PV(2), [Pq(a) for a in rows(0)] + QK(1) + [OPq(a) for a in rows(3)])
            seq += _interleave(PV(1), QK(0) + [OPq(a) for a in rows(2)])
            seq += PV(0) + [OPq(a) for a in rows(1)] + [OPq(a) for a in rows(0)]
        for _, f in seq:
            f()


    with _scope("head"):
        for hh in range(HPS):
            head(hh)

    @pl.when(step == NSTEP - 1)
    def _epilogue():
      with _scope("epilogue"):
        cp_oa((NSTEP - 2) * RST).wait()
        cp_oa((NSTEP - 1) * RST).start()
        cp_oa((NSTEP - 1) * RST).wait()
        for c in range(S // PC):
            cp_ob(c).wait()


@jax.jit
def pallas_concat_heads__sliding_local_dilated__compressed_kv_cla__prompt_kernel(
    A_x, A_wqkv, A_wo, B_x, B_c_kv, B_w_q, B_w_uk, B_w_uv, B_w_o,
):
    any_spec = pl.BlockSpec(memory_space=pl.ANY)
    scratch = [
        pltpu.VMEM((S, M), bf16),
        pltpu.VMEM((M, 3 * M), bf16),
        pltpu.VMEM((M, M), bf16),
        pltpu.VMEM((G, 3 * M, 128), f32),
        pltpu.VMEM((3 * M, M), bf16),
        pltpu.VMEM((M, M), bf16),
        pltpu.VMEM((G, S, 128), f32),
        pltpu.VMEM((G, S + PAD, 128), f32),
        pltpu.VMEM((G, S + PAD, 128), f32),
        pltpu.VMEM((S, M), bf16),
        pltpu.VMEM((S, M), bf16),
        pltpu.VMEM((S, DC), bf16),
        pltpu.VMEM((2, M, D), u32),
        pltpu.VMEM((2, DC, D), u32),
        pltpu.VMEM((2, DC, D), u32),
        pltpu.VMEM((H, D, M), bf16),
        pltpu.VMEM((M, D), bf16),
        pltpu.VMEM((DC, D), bf16),
        pltpu.VMEM((D, DC), bf16),
        pltpu.VMEM((S, D), bf16),
        pltpu.VMEM((S, D), bf16),
        pltpu.VMEM((D, S), bf16),
        pltpu.VMEM((4, 1 * BQ, 128), f32),
        pltpu.VMEM((4, 2 * BQ, 128), f32),
        pltpu.VMEM((4, 3 * BQ, 128), f32),
        pltpu.VMEM((4, 4 * BQ, 128), f32),
        pltpu.VMEM((4, 1 * BQ, 128), f32),
        pltpu.VMEM((4, 2 * BQ, 128), f32),
        pltpu.VMEM((4, 3 * BQ, 128), f32),
        pltpu.VMEM((4, 4 * BQ, 128), f32),
        pltpu.VMEM((S, M), f32),
        pltpu.VMEM((S, M), bf16),
        pltpu.SMEM((2,), jnp.int32),
        pltpu.SemaphoreType.DMA((9 + NA,)),
        pltpu.SemaphoreType.DMA((2, 3)),
        pltpu.SemaphoreType.DMA((1 + S // PC,)),
    ]
    out = pl.pallas_call(
        _kernel,
        grid=(H // HPS,),
        in_specs=[any_spec] * 9,
        out_specs=any_spec,
        out_shape=jax.ShapeDtypeStruct((S, 2 * M), bf16),
        scratch_shapes=scratch,
        compiler_params=pltpu.CompilerParams(
            dimension_semantics=("arbitrary",), vmem_limit_bytes=110 * 1024 * 1024),
    )(A_x.reshape(S, M), A_wqkv, A_wo, B_x.reshape(S, M), B_c_kv.reshape(S, DC),
      B_w_q, B_w_uk, B_w_uv, B_w_o)
    return out.reshape(1, S, 2 * M)
```

```python
import math

import jax
import jax.numpy as jnp
from jax import lax
import jax.experimental.pallas as pl
import jax.experimental.pallas.tpu as pltpu

f32 = jnp.float32
bf16 = jnp.bfloat16
u32 = jnp.uint32

S = 2048
M = 640
G = M // 128
HA = 32
DA = 20
WIN = 8
DIL = 2
PAD = 16
RA = 512
NA = S // RA
AG = 16
H = 32
D = 128
DC = 512
GC = DC // 128
BQ = 512
PC = 256
KC = 256
PVK = 4
HPS = 2
NSTEP = H // HPS
RS = S // H
RST = RS * HPS
LAGC = 192

LOG2E = math.log2(math.e)
QSCALE_A = (DA ** -0.5) * LOG2E
QSCALE_B = (D ** -0.5) * LOG2E
NEG = -1e9 * LOG2E
NT = (((1,), (1,)), ((), ()))
HI_MASK = 0xFFFF0000


def _tree(parts, op):
    parts = list(parts)
    while len(parts) > 1:
        nxt = [op(parts[a], parts[a + 1]) for a in range(0, len(parts) - 1, 2)]
        if len(parts) % 2:
            nxt.append(parts[-1])
        parts = nxt
    return parts[0]


def _fold8(x, op):
    n = x.shape[0] // 8
    return _tree([x[j * 8:(j + 1) * 8] for j in range(n)], op)


def _interleave(heavy, light):
    th = sum(c for c, _ in heavy)
    tl = sum(c for c, _ in light)
    out = []
    ih = il = 0
    dh = dl = 0
    while ih < len(heavy) or il < len(light):
        fh = dh / th if th else 1.0
        fl = dl / tl if tl else 1.0
        if il < len(light) and (ih >= len(heavy) or fl <= fh):
            out.append(light[il])
            dl += light[il][0]
            il += 1
        else:
            out.append(heavy[ih])
            dh += heavy[ih][0]
            ih += 1
    return out


def _pk(x):
    return pltpu.bitcast(x, u32)


def _up(x):
    return pltpu.bitcast(x, bf16)


def _half(r0, n):
    if isinstance(r0, int):
        return pl.ds(r0 // 2, n // 2)
    return pl.ds(pl.multiple_of(lax.shift_right_logical(r0, 1), 8), n // 2)


def _mm(a, b):
    return jnp.dot(a, b, preferred_element_type=f32)


def _mm_nt(a, b):
    return lax.dot_general(a, b, NT, preferred_element_type=f32)


def _kernel(ax_hbm, aw_hbm, awo_hbm, bx_hbm, bc_hbm, wq_hbm, wk_hbm, wv_hbm, wo_hbm,
            out_hbm,
            ax_s, aw_s, awo_s, t_s, wt_s, wop_s, qa_s, ka_s, va_s, oa_s,
            bx_s, bc_s, wq32, wk32, wv32, wo_s, wqh, wkh, wvth,
            q_s, k_s, vt_s, acc_ref, ob_s,
            z_s, sem_in, sem_w, sem_out, *sbufs):
    step = pl.program_id(0)

    def lanes(g):
        return pl.ds(g * 128, 128)

    def cp_aw(sec):
        return [pltpu.make_async_copy(aw_hbm.at[:, pl.ds(sec * M, M)], aw_s.at[:, pl.ds(sec * M, M)],
                                      sem_in.at[sec])]

    def cp_ax(c):
        return [pltpu.make_async_copy(ax_hbm.at[pl.ds(c * RA, RA), lanes(g)],
                                      ax_s.bitcast(bf16).at[g, pl.ds(c * RA, RA)],
                                      sem_in.at[3 + c]) for g in range(G)]

    cp_awo = [pltpu.make_async_copy(awo_hbm.at[:, lanes(g)], awo_s.bitcast(bf16).at[g], sem_in.at[3 + NA])
              for g in range(G)]
    cp_b = (
        [pltpu.make_async_copy(bx_hbm.at[:, lanes(g)], bx_s.bitcast(bf16).at[g], sem_in.at[4 + NA])
         for g in range(G)]
        + [pltpu.make_async_copy(bc_hbm.at[:, lanes(g)], bc_s.bitcast(bf16).at[g], sem_in.at[4 + NA])
           for g in range(GC)]
        + [pltpu.make_async_copy(wo_hbm.at[:, :, lanes(g)], wo_s.bitcast(bf16).at[g], sem_in.at[4 + NA])
           for g in range(G)]
    )

    def start(cps):
        for cp in cps:
            cp.start()

    def wait(cps):
        for cp in cps:
            cp.wait()

    def cp_w(j, slot):
        return [
            pltpu.make_async_copy(src.bitcast(u32).at[:, j, :], dst.at[slot], sem_w.at[slot, i])
            for i, (src, dst) in enumerate(((wq_hbm, wq32), (wk_hbm, wk32), (wv_hbm, wv32)))
        ]

    def cp_oa(r0):
        return pltpu.make_async_copy(oa_s.at[pl.ds(r0, RST)], out_hbm.at[pl.ds(r0, RST), pl.ds(0, M)],
                                     sem_out.at[0])

    def cp_ob(c):
        return pltpu.make_async_copy(ob_s.at[pl.ds(c * PC, PC)], out_hbm.at[pl.ds(c * PC, PC), pl.ds(M, M)],
                                     sem_out.at[1 + c])

    def unpack(w32, par, slot):
        w = w32[slot]
        w = (w & jnp.uint32(HI_MASK)) if par else (w << 16)
        return pltpu.bitcast(w, f32)

    def ext_q(par, slot):
        wqh[par] = _pk(unpack(wq32, par, slot).astype(bf16))

    def ext_k(par, slot):
        wkh[par] = _pk(unpack(wk32, par, slot).astype(bf16))

    def ext_v(par, slot):
        w = unpack(wv32, par, slot)
        for g in range(GC):
            wvth[par * GC + g] = _pk(w[g * 128:(g + 1) * 128, :].T.astype(bf16))

    def prep_t(sec):
        for cb in range(G):
            c0 = sec * M + cb * 128
            for g in range(G):
                t_s[g, c0:c0 + 128, :] = aw_s[g * 128:(g + 1) * 128, c0:c0 + 128].astype(f32).T

    def prep_g(sec):
        for d in range(DA):
            for g in range(G):
                wt_s[g, _half(sec * M + d * HA, HA), :] = _pk(
                    t_s[g, pl.ds(sec * M + d, HA, stride=DA), :].astype(bf16))

    def prep_w(sec):
        prep_t(sec)
        prep_g(sec)

    def prep_wo():
        for e in range(DA // 2):
            for g in range(G):
                w = awo_s[g, pl.ds(e, HA, stride=DA // 2), :]
                lo = pltpu.bitcast(w << 16, f32)
                hi = pltpu.bitcast(w & jnp.uint32(HI_MASK), f32)
                wop_s[g, _half(2 * e * HA, 2 * HA), :] = _pk(jnp.concatenate([lo, hi], axis=0).astype(bf16))

    def a_proj(rbase, secs):
        for sec in secs:
            for sub in range(RA // PC):
                r0 = rbase + sub * PC
                for n in range(G):
                    n0 = sec * M + n * 128
                    t = _tree([_mm_nt(_up(ax_s[g, _half(r0, PC), :]), _up(wt_s[g, _half(n0, 128), :]))
                               for g in range(G)], jnp.add)
                    if sec == 0:
                        qa_s[n, pl.ds(r0, PC), :] = t * QSCALE_A
                    elif sec == 1:
                        ka_s[n, pl.ds(r0 + PAD, PC), :] = t
                    else:
                        va_s[n, pl.ds(r0 + PAD, PC), :] = t

    def a_attn(rbase, never):
        outs = []
        prev = None
        for sub in range(RS // AG):
            rr = rbase + sub * AG
            q = [qa_s[g, pl.ds(rr, AG), :] for g in range(G)]
            if prev is not None:
                q = [jnp.where(never, prev, q[g]) for g in range(G)]
            lg = []
            for w in range(WIN):
                acc = _tree([q[g] * ka_s[g, pl.ds(rr + (PAD - DIL * w), AG), :] for g in range(G)], jnp.add)
                acc = acc + pltpu.roll(acc, 64, 1)
                acc = acc + pltpu.roll(acc, 32, 1)
                if w > 0 and sub * AG < PAD:
                    rowid = rr + lax.broadcasted_iota(jnp.int32, (AG, 128), 0)
                    acc = jnp.where(rowid >= DIL * w, acc, NEG)
                lg.append(acc)
            m = _tree(lg, jnp.maximum)
            e = [jnp.exp2(x - m) for x in lg]
            inv = pl.reciprocal(_tree(e, jnp.add), approx=False)
            og = []
            for g in range(G):
                acc = _tree([e[w] * va_s[g, pl.ds(rr + (PAD - DIL * w), AG), :] for w in range(WIN)], jnp.add)
                og.append(acc * inv)
            prev = og[-1]
            outs.append(jnp.concatenate(og, axis=1))
        return jnp.concatenate(outs, axis=0).astype(bf16)

    @pl.when(step == 0)
    def _prologue():
        start(cp_aw(0))
        start(cp_ax(0))
        start(cp_aw(1))
        start(cp_ax(1))
        start(cp_aw(2))
        z_s[0] = 0
        z_s[1] = 0
        zero = jnp.zeros((PAD, 128), f32)
        for g in range(G):
            ka_s[g, 0:PAD, :] = zero
            va_s[g, 0:PAD, :] = zero
        acc_ref[...] = jnp.zeros_like(acc_ref)
        wait(cp_aw(0))
        for c in range(2, NA):
            start(cp_ax(c))
        start(cp_awo)
        prep_t(0)
        wait(cp_ax(0))
        prep_g(0)
        a_proj(0, (0,))
        wait(cp_aw(1))
        wait(cp_ax(1))
        start(cp_w(0, 0))
        start(cp_b)
        a_proj(RA, (0,))
        prep_w(1)
        a_proj(0, (1,))
        wait(cp_aw(2))
        wait(cp_ax(2))
        wait(cp_awo)
        wait(cp_ax(3))
        a_proj(2 * RA, (0,))
        prep_wo()
        a_proj(3 * RA, (0,))
        prep_w(2)
        a_proj(0, (2,))

        def body(c, carry):
            a_proj(pl.multiple_of(c * RA, RA), (1, 2))
            return carry
        lax.fori_loop(1, NA, body, 0)
        wait(cp_b)

    slot = step & 1
    wait(cp_w(step, slot))

    @pl.when(step >= 1)
    def _():
        cp_oa(pl.multiple_of((step - 1) * RST, RST)).wait()

    @pl.when(step + 1 < NSTEP)
    def _():
        start(cp_w(step + 1, 1 - slot))

    zs = z_s[0]
    zl = z_s[1]
    never = zs != 0
    row = lax.broadcasted_iota(jnp.int32, (128, 128), 0)
    col = lax.broadcasted_iota(jnp.int32, (128, 128), 1)
    tri = row <= col

    obs = [{} for _ in range(HPS)]
    tokens = []
    clock = [0]

    def pub(r):
        tokens.append((clock[0], r[0:1, 0:128]))

    def token(lag):
        cand = [t for c0, t in tokens if c0 <= clock[0] - lag]
        return cand[-1] if cand else None

    def head(hh):
        h = step * HPS + hh
        sb = sbufs[4 * hh:4 * hh + 4]
        ra = pl.multiple_of(h * RS, RS)
        pm = {}
        mx = {}
        ot = {}
        ls = {}
        ob = obs[hh]
        oa = {}

        def Pq(a):
            def f():
                r = _tree([_mm(_up(bx_s[g, _half(a, PC), :]), _up(wqh[hh, _half(g * 128, 128), :]))
                           for g in range(G)], jnp.add)
                q_s[hh, _half(a, PC), :] = _pk((r * QSCALE_B).astype(bf16))
                pub(r)
            return (PC // 16 * G, f)

        def Pk(a):
            def f():
                r = _tree([_mm(_up(bc_s[g, _half(a, PC), :]), _up(wkh[hh, _half(g * 128, 128), :]))
                           for g in range(GC)], jnp.add)
                k_s[hh, _half(a, PC), :] = _pk(r.astype(bf16))
                pub(r)
            return (PC // 16 * GC, f)

        def Pv(a):
            def f():
                for j in range(a // 128, (a + PC) // 128):
                    r = _tree([_mm_nt(_up(wvth[hh * GC + g]), _up(bc_s[g, _half(j * 128, 128), :]))
                               for g in range(GC)], jnp.add)
                    vt_s[hh * 16 + j] = _pk(r.astype(bf16))
                pub(r)
            return (PC // 16 * GC, f)

        def QKq(i, k0, k1, t0):
            lo = i * BQ

            def f():
                r = _mm_nt(_up(k_s[hh, _half(k0, k1 - k0), :]),
                           _up(q_s[hh, _half(lo + t0 * 128, BQ - t0 * 128), :]))
                pub(r)
                for t in range(t0, 4):
                    c = i * 4 + t
                    for j in range(k0 // 128, k1 // 128):
                        tile = r[j * 128 - k0:(j + 1) * 128 - k0, (t - t0) * 128:(t - t0 + 1) * 128]
                        if j == c:
                            tile = jnp.where(tri, tile, NEG)
                        sb[i][zs + t, j * 128:(j + 1) * 128, :] = tile
                        pm.setdefault(c, []).append(_fold8(tile, jnp.maximum))
            return ((k1 - k0) // 16 * (4 - t0), f)

        def QK(i):
            lo = i * BQ
            qs = []
            k0 = 0
            while k0 < lo + 128:
                k1 = min(k0 + KC, lo + 128)
                qs.append(QKq(i, k0, k1, 0))
                k0 = k1
            for u in range(1, 4):
                qs.append(QKq(i, lo + u * 128, lo + (u + 1) * 128, u))
            return qs

        def PVq(c, j0, j1):
            def f():
                if c not in mx:
                    mx[c] = jnp.max(_tree(pm.pop(c), jnp.maximum), axis=0, keepdims=True)
                m = mx[c]
                tok = token(LAGC)
                if tok is not None:
                    m = jnp.where(never, tok, m)
                ps = [jnp.exp2(sb[c // 4][zl + c % 4, j * 128:(j + 1) * 128, :] - m) for j in range(j0, j1)]
                lsum = _tree([_fold8(p, jnp.add) for p in ps], jnp.add)
                ls[c] = lsum if c not in ls else ls[c] + lsum
                o = _tree([_mm(_up(vt_s[hh * 16 + j]), p.astype(bf16)) for j, p in zip(range(j0, j1), ps)],
                          jnp.add)
                pub(o)
                ot[c] = o if c not in ot else ot[c] + o
                if j1 == c + 1:
                    l = jnp.sum(ls.pop(c), axis=0, keepdims=True)
                    ob[c] = (ot.pop(c) * pl.reciprocal(l, approx=False)).T
            return ((j1 - j0) * 8, f)

        def PV(i):
            qs = []
            for t in range(4):
                c = i * 4 + t
                for j0 in range(0, c + 1, PVK):
                    qs.append(PVq(c, j0, min(j0 + PVK, c + 1)))
            return qs

        def OPq(a):
            def f():
                cs = range(a // 128, (a + PC) // 128)
                os_ = [jnp.concatenate([obs[u].pop(c) for c in cs], axis=0).astype(bf16) for u in range(HPS)]
                for g in range(G):
                    new = acc_ref[a:a + PC, g * 128:(g + 1) * 128] + _tree(
                        [_mm(os_[u], _up(wo_s[g, step * HPS + u])) for u in range(HPS)], jnp.add)
                    acc_ref[a:a + PC, g * 128:(g + 1) * 128] = new
                    if g == 0:
                        pub(new)
                    ob_s[a:a + PC, g * 128:(g + 1) * 128] = new.astype(bf16)

                @pl.when(step == NSTEP - 1)
                def _():
                    cp_ob(a // PC).start()
            return (PC // 16 * G * HPS, f)

        def do(fn, *args):
            return (0, lambda: fn(*args))

        def Aattn():
            oa[0] = a_attn(ra, never)

        def Aout():
            o = oa.pop(0)
            for g in range(G):
                oa_s[pl.ds(ra, RS), g * 128:(g + 1) * 128] = _mm(o, _up(wop_s[g])).astype(bf16)
            if hh == HPS - 1:
                cp_oa(pl.multiple_of(step * RST, RST)).start()

        def rows(i):
            return range(i * BQ, (i + 1) * BQ, PC)

        return dict(
            ext=[do(ext_q, hh, slot), do(ext_k, hh, slot), do(ext_v, hh, slot), do(Aattn)],
            aout=[do(Aout)],
            pq=lambda i: [Pq(a) for a in rows(i)],
            op=lambda i: [OPq(a) for a in rows(i)],
            QK=QK, PV=PV,
            pk=[Pk(a) for a in range(0, S, PC)],
            pv=[Pv(a) for a in range(0, S, PC)])

    A = head(0)
    B = head(1)
    pre_a = A['pq'](3) + A['pk'] + A['aout'] + A['QK'](3) + A['pq'](2) + A['pv']
    pre_b = B['ext'] + B['pq'](3) + B['pk'] + B['aout'] + B['QK'](3) + B['pq'](2) + B['pv']
    seq = A['ext'] + pre_a
    seq += _interleave(A['PV'](3), A['pq'](1) + A['QK'](2))
    seq += _interleave(A['PV'](2), A['pq'](0) + A['QK'](1) + pre_b[:5])
    seq += _interleave(A['PV'](1), A['QK'](0) + pre_b[5:8])
    seq += _interleave(A['PV'](0), pre_b[8:11])
    seq += pre_b[11:]
    seq += _interleave(B['PV'](3), B['QK'](2) + B['pq'](1))
    seq += _interleave(B['PV'](2), B['pq'](0) + B['QK'](1) + B['op'](3))
    seq += _interleave(B['PV'](1), B['QK'](0) + B['op'](2))
    seq += B['PV'](0) + B['op'](1) + B['op'](0)
    for cost, f in seq:
        f()
        clock[0] += cost

    @pl.when(step == NSTEP - 1)
    def _epilogue():
        cp_oa((NSTEP - 1) * RST).wait()
        for c in range(S // PC):
            cp_ob(c).wait()


@jax.jit
def pallas_concat_heads__sliding_local_dilated__compressed_kv_cla__prompt_kernel(
    A_x: jax.Array,
    A_wqkv: jax.Array,
    A_wo: jax.Array,
    B_x: jax.Array,
    B_c_kv: jax.Array,
    B_w_q: jax.Array,
    B_w_uk: jax.Array,
    B_w_uv: jax.Array,
    B_w_o: jax.Array,
):
    any_spec = pl.BlockSpec(memory_space=pl.ANY)
    scratch = [
        pltpu.VMEM((G, S // 2, 128), u32),
        pltpu.VMEM((M, 3 * M), bf16),
        pltpu.VMEM((G, M // 2, 128), u32),
        pltpu.VMEM((G, 3 * M, 128), f32),
        pltpu.VMEM((G, 3 * M // 2, 128), u32),
        pltpu.VMEM((G, M // 2, 128), u32),
        pltpu.VMEM((G, S, 128), f32),
        pltpu.VMEM((G, S + PAD, 128), f32),
        pltpu.VMEM((G, S + PAD, 128), f32),
        pltpu.VMEM((S, M), bf16),
        pltpu.VMEM((G, S // 2, 128), u32),
        pltpu.VMEM((GC, S // 2, 128), u32),
        pltpu.VMEM((2, M, D), u32),
        pltpu.VMEM((2, DC, D), u32),
        pltpu.VMEM((2, DC, D), u32),
        pltpu.VMEM((G, H, D // 2, 128), u32),
        pltpu.VMEM((HPS, M // 2, D), u32),
        pltpu.VMEM((HPS, DC // 2, D), u32),
        pltpu.VMEM((HPS * GC, D // 2, 128), u32),
        pltpu.VMEM((HPS, S // 2, D), u32),
        pltpu.VMEM((HPS, S // 2, D), u32),
        pltpu.VMEM((HPS * S // 128, D // 2, 128), u32),
        pltpu.VMEM((S, M), f32),
        pltpu.VMEM((S, M), bf16),
        pltpu.SMEM((2,), jnp.int32),
        pltpu.SemaphoreType.DMA((5 + NA,)),
        pltpu.SemaphoreType.DMA((2, 3)),
        pltpu.SemaphoreType.DMA((1 + S // PC,)),
    ]
    scratch += [pltpu.VMEM((4, (i + 1) * BQ, 128), f32) for _ in range(HPS) for i in range(4)]
    out = pl.pallas_call(
        _kernel,
        grid=(NSTEP,),
        in_specs=[any_spec] * 9,
        out_specs=any_spec,
        out_shape=jax.ShapeDtypeStruct((S, 2 * M), bf16),
        scratch_shapes=scratch,
        compiler_params=pltpu.CompilerParams(
            dimension_semantics=("arbitrary",), vmem_limit_bytes=110 * 1024 * 1024),
    )(A_x.reshape(S, M), A_wqkv, A_wo, B_x.reshape(S, M), B_c_kv.reshape(S, DC),
      B_w_q, B_w_uk, B_w_uv, B_w_o)
    return out.reshape(1, S, 2 * M)
```

```python
import math

import jax
import jax.numpy as jnp
from jax import lax
import jax.experimental.pallas as pl
import jax.experimental.pallas.tpu as pltpu

f32 = jnp.float32
bf16 = jnp.bfloat16
u32 = jnp.uint32

S = 2048
M = 640
G = M // 128
HA = 32
DA = 20
WIN = 8
DIL = 2
PAD = 16
RA = 512
NA = S // RA
AG = 16
H = 32
D = 128
DC = 512
GC = DC // 128
BQ = 512
PC = 256
KC = 256
PVK = 4
HPS = 2
NSTEP = H // HPS
RS = S // H
RST = RS * HPS
LAGC = 192

LOG2E = math.log2(math.e)
QSCALE_A = (DA ** -0.5) * LOG2E
QSCALE_B = (D ** -0.5) * LOG2E
NEG = -1e9 * LOG2E
NT = (((1,), (1,)), ((), ()))
HI_MASK = 0xFFFF0000


def _tree(parts, op):
    parts = list(parts)
    while len(parts) > 1:
        nxt = [op(parts[a], parts[a + 1]) for a in range(0, len(parts) - 1, 2)]
        if len(parts) % 2:
            nxt.append(parts[-1])
        parts = nxt
    return parts[0]


def _fold8(x, op):
    n = x.shape[0] // 8
    return _tree([x[j * 8:(j + 1) * 8] for j in range(n)], op)


def _interleave(heavy, light):
    th = sum(c for c, _ in heavy)
    tl = sum(c for c, _ in light)
    out = []
    ih = il = 0
    dh = dl = 0
    while ih < len(heavy) or il < len(light):
        fh = dh / th if th else 1.0
        fl = dl / tl if tl else 1.0
        if il < len(light) and (ih >= len(heavy) or fl <= fh):
            out.append(light[il])
            dl += light[il][0]
            il += 1
        else:
            out.append(heavy[ih])
            dh += heavy[ih][0]
            ih += 1
    return out


def _pk(x):
    return pltpu.bitcast(x, u32)


def _up(x):
    return pltpu.bitcast(x, bf16)


def _half(r0, n):
    if isinstance(r0, int):
        return pl.ds(r0 // 2, n // 2)
    return pl.ds(pl.multiple_of(lax.shift_right_logical(r0, 1), 8), n // 2)


def _mm(a, b):
    return jnp.dot(a, b, preferred_element_type=f32)


def _mm_nt(a, b):
    return lax.dot_general(a, b, NT, preferred_element_type=f32)


def _kernel(ax_hbm, aw_hbm, awo_hbm, bx_hbm, bc_hbm, wq_hbm, wk_hbm, wv_hbm, wo_hbm,
            out_hbm,
            ax_s, aw_s, awo_s, t_s, wt_s, wop_s, qa_s, ka_s, va_s, oa_s,
            bx_s, bc_s, w32, wo_s, wqh, wkh, wvth,
            q_s, k_s, vt_s, acc_ref, ob_s,
            z_s, sem_in, sem_w, sem_out, *sbufs):
    step = pl.program_id(0)

    def lanes(g):
        return pl.ds(g * 128, 128)

    def cp_aw(sec):
        return [pltpu.make_async_copy(aw_hbm.at[:, pl.ds(sec * M, M)], aw_s.at[:, pl.ds(sec * M, M)],
                                      sem_in.at[sec])]

    def cp_ax(c):
        return [pltpu.make_async_copy(ax_hbm.at[pl.ds(c * RA, RA), lanes(g)],
                                      ax_s.bitcast(bf16).at[g, pl.ds(c * RA, RA)],
                                      sem_in.at[3 + c]) for g in range(G)]

    cp_awo = [pltpu.make_async_copy(awo_hbm.at[:, lanes(g)], awo_s.bitcast(bf16).at[g], sem_in.at[3 + NA])
              for g in range(G)]
    cp_b = (
        [pltpu.make_async_copy(bx_hbm.at[:, lanes(g)], bx_s.bitcast(bf16).at[g], sem_in.at[4 + NA])
         for g in range(G)]
        + [pltpu.make_async_copy(bc_hbm.at[:, lanes(g)], bc_s.bitcast(bf16).at[g], sem_in.at[4 + NA])
           for g in range(GC)]
        + [pltpu.make_async_copy(wo_hbm.at[:, :, lanes(g)], wo_s.bitcast(bf16).at[g], sem_in.at[4 + NA])
           for g in range(G)]
    )

    def start(cps):
        for cp in cps:
            cp.start()

    def wait(cps):
        for cp in cps:
            cp.wait()

    def cp_w(j, slot):
        return [
            pltpu.make_async_copy(src.bitcast(u32).at[:, j, :], w32.at[slot, pl.ds(r0, n)], sem_w.at[slot])
            for src, r0, n in ((wq_hbm, 0, M), (wk_hbm, M, DC), (wv_hbm, M + DC, DC))
        ]

    def wait_w(slot):
        pltpu.make_async_copy(w32.at[slot], w32.at[slot], sem_w.at[slot]).wait()

    def cp_oa(r0):
        return pltpu.make_async_copy(oa_s.at[pl.ds(r0, RST)], out_hbm.at[pl.ds(r0, RST), pl.ds(0, M)],
                                     sem_out.at[0])

    def cp_ob(c):
        return pltpu.make_async_copy(ob_s.at[pl.ds(c * PC, PC)], out_hbm.at[pl.ds(c * PC, PC), pl.ds(M, M)],
                                     sem_out.at[1])

    def unpack(r0, n, par, slot):
        w = w32[slot, r0:r0 + n, :]
        w = (w & jnp.uint32(HI_MASK)) if par else (w << 16)
        return pltpu.bitcast(w, f32)

    def ext_q(par, slot):
        wqh[par] = _pk(unpack(0, M, par, slot).astype(bf16))

    def ext_k(par, slot):
        wkh[par] = _pk(unpack(M, DC, par, slot).astype(bf16))

    def ext_v(par, slot):
        w = unpack(M + DC, DC, par, slot)
        for g in range(GC):
            wvth[par * GC + g] = _pk(w[g * 128:(g + 1) * 128, :].T.astype(bf16))

    def prep_t(sec):
        for cb in range(G):
            c0 = sec * M + cb * 128
            for g in range(G):
                t_s[g, c0:c0 + 128, :] = aw_s[g * 128:(g + 1) * 128, c0:c0 + 128].astype(f32).T

    def prep_g(sec):
        for d in range(DA):
            for g in range(G):
                wt_s[g, _half(sec * M + d * HA, HA), :] = _pk(
                    t_s[g, pl.ds(sec * M + d, HA, stride=DA), :].astype(bf16))

    def prep_w(sec):
        prep_t(sec)
        prep_g(sec)

    def prep_wo():
        for e in range(DA // 2):
            for g in range(G):
                w = awo_s[g, pl.ds(e, HA, stride=DA // 2), :]
                lo = pltpu.bitcast(w << 16, f32)
                hi = pltpu.bitcast(w & jnp.uint32(HI_MASK), f32)
                wop_s[g, _half(2 * e * HA, 2 * HA), :] = _pk(jnp.concatenate([lo, hi], axis=0).astype(bf16))

    def a_proj(rbase, secs):
        for sec in secs:
            for sub in range(RA // PC):
                r0 = rbase + sub * PC
                for n in range(G):
                    n0 = sec * M + n * 128
                    t = _tree([_mm_nt(_up(ax_s[g, _half(r0, PC), :]), _up(wt_s[g, _half(n0, 128), :]))
                               for g in range(G)], jnp.add)
                    if sec == 0:
                        qa_s[n, pl.ds(r0, PC), :] = t * QSCALE_A
                    elif sec == 1:
                        ka_s[n, pl.ds(r0 + PAD, PC), :] = t
                    else:
                        va_s[n, pl.ds(r0 + PAD, PC), :] = t

    def a_attn(rbase, never):
        outs = []
        prev = None
        for sub in range(RS // AG):
            rr = rbase + sub * AG
            q = [qa_s[g, pl.ds(rr, AG), :] for g in range(G)]
            if prev is not None:
                q = [jnp.where(never, prev, q[g]) for g in range(G)]
            lg = []
            for w in range(WIN):
                acc = _tree([q[g] * ka_s[g, pl.ds(rr + (PAD - DIL * w), AG), :] for g in range(G)], jnp.add)
                acc = acc + pltpu.roll(acc, 64, 1)
                acc = acc + pltpu.roll(acc, 32, 1)
                if w > 0 and sub * AG < PAD:
                    rowid = rr + lax.broadcasted_iota(jnp.int32, (AG, 128), 0)
                    acc = jnp.where(rowid >= DIL * w, acc, NEG)
                lg.append(acc)
            m = _tree(lg, jnp.maximum)
            e = [jnp.exp2(x - m) for x in lg]
            inv = pl.reciprocal(_tree(e, jnp.add), approx=False)
            og = []
            for g in range(G):
                acc = _tree([e[w] * va_s[g, pl.ds(rr + (PAD - DIL * w), AG), :] for w in range(WIN)], jnp.add)
                og.append(acc * inv)
            prev = og[-1]
            outs.append(jnp.concatenate(og, axis=1))
        return jnp.concatenate(outs, axis=0).astype(bf16)

    @pl.when(step == 0)
    def _prologue():
        start(cp_aw(0))
        start(cp_ax(0))
        z_s[0] = 0
        z_s[1] = 0
        zero = jnp.zeros((PAD, 128), f32)
        for g in range(G):
            ka_s[g, 0:PAD, :] = zero
            va_s[g, 0:PAD, :] = zero
        acc_ref[...] = jnp.zeros_like(acc_ref)
        wait(cp_aw(0))
        start(cp_aw(1))
        start(cp_ax(1))
        start(cp_aw(2))
        for c in range(2, NA):
            start(cp_ax(c))
        start(cp_awo)
        prep_w(0)
        wait(cp_ax(0))
        a_proj(0, (0,))
        wait(cp_aw(1))
        wait(cp_ax(1))
        start(cp_w(0, 0))
        start(cp_b)
        a_proj(RA, (0,))
        prep_w(1)
        a_proj(0, (1,))
        wait(cp_aw(2))
        wait(cp_ax(2))
        wait(cp_awo)
        wait(cp_ax(3))
        a_proj(2 * RA, (0,))
        prep_wo()
        a_proj(3 * RA, (0,))
        prep_w(2)
        a_proj(0, (2,))

        def body(c, carry):
            a_proj(pl.multiple_of(c * RA, RA), (1, 2))
            return carry
        lax.fori_loop(1, NA, body, 0)
        wait(cp_b)

    slot = step & 1
    wait_w(slot)

    @pl.when(step >= 1)
    def _():
        cp_oa(pl.multiple_of((step - 1) * RST, RST)).wait()

    def prefetch_w():
        @pl.when(step + 1 < NSTEP)
        def _():
            start(cp_w(step + 1, 1 - slot))

    zs = z_s[0]
    zl = z_s[1]
    never = zs != 0
    row = lax.broadcasted_iota(jnp.int32, (128, 128), 0)
    col = lax.broadcasted_iota(jnp.int32, (128, 128), 1)
    tri = row <= col

    obs = [{} for _ in range(HPS)]
    tokens = []
    clock = [0]

    def pub(r):
        tokens.append((clock[0], r[0:1, 0:128]))

    def token(lag):
        cand = [t for c0, t in tokens if c0 <= clock[0] - lag]
        return cand[-1] if cand else None

    def head(hh):
        h = step * HPS + hh
        sb = sbufs[4 * hh:4 * hh + 4]
        ra = pl.multiple_of(h * RS, RS)
        pm = {}
        mx = {}
        ot = {}
        ls = {}
        ob = obs[hh]
        oa = {}

        def Pq(a):
            def f():
                r = _tree([_mm(_up(bx_s[g, _half(a, PC), :]), _up(wqh[hh, _half(g * 128, 128), :]))
                           for g in range(G)], jnp.add)
                q_s[hh, _half(a, PC), :] = _pk((r * QSCALE_B).astype(bf16))
                pub(r)
            return (PC // 16 * G, f)

        def Pk(a):
            def f():
                r = _tree([_mm(_up(bc_s[g, _half(a, PC), :]), _up(wkh[hh, _half(g * 128, 128), :]))
                           for g in range(GC)], jnp.add)
                k_s[hh, _half(a, PC), :] = _pk(r.astype(bf16))
                pub(r)
            return (PC // 16 * GC, f)

        def Pv(a):
            def f():
                for j in range(a // 128, (a + PC) // 128):
                    r = _tree([_mm_nt(_up(wvth[hh * GC + g]), _up(bc_s[g, _half(j * 128, 128), :]))
                               for g in range(GC)], jnp.add)
                    vt_s[hh * 16 + j] = _pk(r.astype(bf16))
                pub(r)
            return (PC // 16 * GC, f)

        def QKq(i, k0, k1, t0):
            lo = i * BQ

            def f():
                r = _mm_nt(_up(k_s[hh, _half(k0, k1 - k0), :]),
                           _up(q_s[hh, _half(lo + t0 * 128, BQ - t0 * 128), :]))
                pub(r)
                for t in range(t0, 4):
                    c = i * 4 + t
                    for j in range(k0 // 128, k1 // 128):
                        tile = r[j * 128 - k0:(j + 1) * 128 - k0, (t - t0) * 128:(t - t0 + 1) * 128]
                        if j == c:
                            tile = jnp.where(tri, tile, NEG)
                        sb[i][zs + t, j * 128:(j + 1) * 128, :] = tile
                        pm.setdefault(c, []).append(_fold8(tile, jnp.maximum))
            return ((k1 - k0) // 16 * (4 - t0), f)

        def QK(i):
            lo = i * BQ
            qs = []
            k0 = 0
            while k0 < lo + 128:
                k1 = min(k0 + KC, lo + 128)
                qs.append(QKq(i, k0, k1, 0))
                k0 = k1
            for u in range(1, 4):
                qs.append(QKq(i, lo + u * 128, lo + (u + 1) * 128, u))
            return qs

        def PVq(c, j0, j1):
            def f():
                if c not in mx:
                    mx[c] = jnp.max(_tree(pm.pop(c), jnp.maximum), axis=0, keepdims=True)
                m = mx[c]
                tok = token(LAGC)
                if tok is not None:
                    m = jnp.where(never, tok, m)
                ps = [jnp.exp2(sb[c // 4][zl + c % 4, j * 128:(j + 1) * 128, :] - m) for j in range(j0, j1)]
                lsum = _tree([_fold8(p, jnp.add) for p in ps], jnp.add)
                ls[c] = lsum if c not in ls else ls[c] + lsum
                o = _tree([_mm(_up(vt_s[hh * 16 + j]), p.astype(bf16)) for j, p in zip(range(j0, j1), ps)],
                          jnp.add)
                pub(o)
                ot[c] = o if c not in ot else ot[c] + o
                if j1 == c + 1:
                    l = jnp.sum(ls.pop(c), axis=0, keepdims=True)
                    ob[c] = (ot.pop(c) * pl.reciprocal(l, approx=False)).T
            return ((j1 - j0) * 8, f)

        def PV(i):
            qs = []
            for t in range(4):
                c = i * 4 + t
                for j0 in range(0, c + 1, PVK):
                    qs.append(PVq(c, j0, min(j0 + PVK, c + 1)))
            return qs

        def OPq(a):
            def f():
                cs = range(a // 128, (a + PC) // 128)
                os_ = [jnp.concatenate([obs[u].pop(c) for c in cs], axis=0).astype(bf16) for u in range(HPS)]
                for g in range(G):
                    new = acc_ref[a:a + PC, g * 128:(g + 1) * 128] + _tree(
                        [_mm(os_[u], _up(wo_s[g, step * HPS + u])) for u in range(HPS)], jnp.add)
                    acc_ref[a:a + PC, g * 128:(g + 1) * 128] = new
                    if g == 0:
                        pub(new)
                    ob_s[a:a + PC, g * 128:(g + 1) * 128] = new.astype(bf16)

                @pl.when(step == NSTEP - 1)
                def _():
                    cp_ob(a // PC).start()
            return (PC // 16 * G * HPS, f)

        def do(fn, *args):
            return (0, lambda: fn(*args))

        def Aattn():
            oa[0] = a_attn(ra, never)

        def Aout():
            o = oa.pop(0)
            for g in range(G):
                oa_s[pl.ds(ra, RS), g * 128:(g + 1) * 128] = _mm(o, _up(wop_s[g])).astype(bf16)
            if hh == HPS - 1:
                cp_oa(pl.multiple_of(step * RST, RST)).start()

        def rows(i):
            return range(i * BQ, (i + 1) * BQ, PC)

        return dict(
            ext=[do(ext_q, hh, slot), do(ext_k, hh, slot), do(ext_v, hh, slot), do(Aattn)],
            aout=[do(Aout)],
            pq=lambda i: [Pq(a) for a in rows(i)],
            op=lambda i: [OPq(a) for a in rows(i)],
            QK=QK, PV=PV,
            pk=[Pk(a) for a in range(0, S, PC)],
            pv=[Pv(a) for a in range(0, S, PC)])

    A = head(0)
    B = head(1)
    pre_a = A['pq'](3) + A['pk'] + A['aout'] + A['QK'](3) + A['pq'](2) + A['pv']
    pre_b = [(0, prefetch_w)] + B['ext'] + B['pq'](3) + B['pk'] + B['aout'] + B['QK'](3) + B['pq'](2) + B['pv']
    seq = A['ext'] + pre_a
    seq += _interleave(A['PV'](3), A['pq'](1) + A['QK'](2))
    seq += _interleave(A['PV'](2), A['pq'](0) + A['QK'](1) + pre_b[:6])
    seq += _interleave(A['PV'](1), A['QK'](0) + pre_b[6:9])
    seq += _interleave(A['PV'](0), pre_b[9:12])
    seq += pre_b[12:]
    seq += _interleave(B['PV'](3), B['QK'](2) + B['pq'](1))
    seq += _interleave(B['PV'](2), B['pq'](0) + B['QK'](1) + B['op'](3))
    seq += _interleave(B['PV'](1), B['QK'](0) + B['op'](2))
    seq += B['PV'](0) + B['op'](1) + B['op'](0)
    for cost, f in seq:
        f()
        clock[0] += cost

    @pl.when(step == NSTEP - 1)
    def _epilogue():
        cp_oa((NSTEP - 1) * RST).wait()
        pltpu.make_async_copy(ob_s, out_hbm.at[:, pl.ds(M, M)], sem_out.at[1]).wait()


@jax.jit
def pallas_concat_heads__sliding_local_dilated__compressed_kv_cla__prompt_kernel(
    A_x: jax.Array,
    A_wqkv: jax.Array,
    A_wo: jax.Array,
    B_x: jax.Array,
    B_c_kv: jax.Array,
    B_w_q: jax.Array,
    B_w_uk: jax.Array,
    B_w_uv: jax.Array,
    B_w_o: jax.Array,
):
    any_spec = pl.BlockSpec(memory_space=pl.ANY)
    scratch = [
        pltpu.VMEM((G, S // 2, 128), u32),
        pltpu.VMEM((M, 3 * M), bf16),
        pltpu.VMEM((G, M // 2, 128), u32),
        pltpu.VMEM((G, 3 * M, 128), f32),
        pltpu.VMEM((G, 3 * M // 2, 128), u32),
        pltpu.VMEM((G, M // 2, 128), u32),
        pltpu.VMEM((G, S, 128), f32),
        pltpu.VMEM((G, S + PAD, 128), f32),
        pltpu.VMEM((G, S + PAD, 128), f32),
        pltpu.VMEM((S, M), bf16),
        pltpu.VMEM((G, S // 2, 128), u32),
        pltpu.VMEM((GC, S // 2, 128), u32),
        pltpu.VMEM((2, M + 2 * DC, D), u32),
        pltpu.VMEM((G, H, D // 2, 128), u32),
        pltpu.VMEM((HPS, M // 2, D), u32),
        pltpu.VMEM((HPS, DC // 2, D), u32),
        pltpu.VMEM((HPS * GC, D // 2, 128), u32),
        pltpu.VMEM((HPS, S // 2, D), u32),
        pltpu.VMEM((HPS, S // 2, D), u32),
        pltpu.VMEM((HPS * S // 128, D // 2, 128), u32),
        pltpu.VMEM((S, M), f32),
        pltpu.VMEM((S, M), bf16),
        pltpu.SMEM((2,), jnp.int32),
        pltpu.SemaphoreType.DMA((5 + NA,)),
        pltpu.SemaphoreType.DMA((2,)),
        pltpu.SemaphoreType.DMA((2,)),
    ]
    scratch += [pltpu.VMEM((4, (i + 1) * BQ, 128), f32) for _ in range(HPS) for i in range(4)]
    out = pl.pallas_call(
        _kernel,
        grid=(NSTEP,),
        in_specs=[any_spec] * 9,
        out_specs=any_spec,
        out_shape=jax.ShapeDtypeStruct((S, 2 * M), bf16),
        scratch_shapes=scratch,
        compiler_params=pltpu.CompilerParams(
            dimension_semantics=("arbitrary",), vmem_limit_bytes=110 * 1024 * 1024),
    )(A_x.reshape(S, M), A_wqkv, A_wo, B_x.reshape(S, M), B_c_kv.reshape(S, DC),
      B_w_q, B_w_uk, B_w_uv, B_w_o)
    return out.reshape(1, S, 2 * M)
```

```python
import math

import jax
import jax.numpy as jnp
from jax import lax
import jax.experimental.pallas as pl
import jax.experimental.pallas.tpu as pltpu

f32 = jnp.float32
bf16 = jnp.bfloat16
u32 = jnp.uint32

S = 2048
M = 640
G = M // 128
HA = 32
DA = 20
WIN = 8
DIL = 2
PAD = 16
RA = 512
NA = S // RA
AG = 16
H = 32
D = 128
DC = 512
GC = DC // 128
BQ = 512
PC = 256
KC = 256
PVK = 4
HPS = 2
NSTEP = H // HPS
RS = S // H
RST = RS * HPS
LAGC = 192

LOG2E = math.log2(math.e)
QSCALE_A = (DA ** -0.5) * LOG2E
QSCALE_B = (D ** -0.5) * LOG2E
NEG = -1e9 * LOG2E
NT = (((1,), (1,)), ((), ()))
HI_MASK = 0xFFFF0000


def _tree(parts, op):
    parts = list(parts)
    while len(parts) > 1:
        nxt = [op(parts[a], parts[a + 1]) for a in range(0, len(parts) - 1, 2)]
        if len(parts) % 2:
            nxt.append(parts[-1])
        parts = nxt
    return parts[0]


def _fold8(x, op):
    n = x.shape[0] // 8
    return _tree([x[j * 8:(j + 1) * 8] for j in range(n)], op)


def _interleave(heavy, light):
    th = sum(c for c, _ in heavy)
    tl = sum(c for c, _ in light)
    out = []
    ih = il = 0
    dh = dl = 0
    while ih < len(heavy) or il < len(light):
        fh = dh / th if th else 1.0
        fl = dl / tl if tl else 1.0
        if il < len(light) and (ih >= len(heavy) or fl <= fh):
            out.append(light[il])
            dl += light[il][0]
            il += 1
        else:
            out.append(heavy[ih])
            dh += heavy[ih][0]
            ih += 1
    return out


def _pk(x):
    return pltpu.bitcast(x, u32)


def _up(x):
    return pltpu.bitcast(x, bf16)


def _half(r0, n):
    if isinstance(r0, int):
        return pl.ds(r0 // 2, n // 2)
    return pl.ds(pl.multiple_of(lax.shift_right_logical(r0, 1), 8), n // 2)


def _mm(a, b):
    return jnp.dot(a, b, preferred_element_type=f32)


def _mm_nt(a, b):
    return lax.dot_general(a, b, NT, preferred_element_type=f32)


def _kernel(ax_hbm, aw_hbm, awo_hbm, bx_hbm, bc_hbm, wq_hbm, wk_hbm, wv_hbm, wo_hbm,
            out_hbm,
            ax_s, aw_s, awo_s, t_s, wt_s, wop_s, qa_s, ka_s, va_s, oa_s,
            bx_s, bc_s, w32, wo_s, wqh, wkh, wvth,
            q_s, k_s, vt_s, acc_ref, ob_s,
            z_s, sem_in, sem_w, sem_out, *sbufs):
    step = pl.program_id(0)

    def lanes(g):
        return pl.ds(g * 128, 128)

    def cp_aw(sec):
        return [pltpu.make_async_copy(aw_hbm.at[:, pl.ds(sec * M, M)], aw_s.at[:, pl.ds(sec * M, M)],
                                      sem_in.at[sec])]

    def cp_ax(c):
        return [pltpu.make_async_copy(ax_hbm.at[pl.ds(c * RA, RA), lanes(g)],
                                      ax_s.bitcast(bf16).at[g, pl.ds(c * RA, RA)],
                                      sem_in.at[3 + c]) for g in range(G)]

    cp_awo = [pltpu.make_async_copy(awo_hbm.at[:, lanes(g)], awo_s.bitcast(bf16).at[g, pl.ds(0, M)],
                                    sem_in.at[3 + NA])
              for g in range(G)]
    cp_b = (
        [pltpu.make_async_copy(bx_hbm.at[:, lanes(g)], bx_s.bitcast(bf16).at[g], sem_in.at[4 + NA])
         for g in range(G)]
        + [pltpu.make_async_copy(bc_hbm.at[:, lanes(g)], bc_s.bitcast(bf16).at[g], sem_in.at[4 + NA])
           for g in range(GC)]
        + [pltpu.make_async_copy(wo_hbm.at[:, :, lanes(g)], wo_s.bitcast(bf16).at[g], sem_in.at[4 + NA])
           for g in range(G)]
    )

    def start(cps):
        for cp in cps:
            cp.start()

    def wait(cps):
        for cp in cps:
            cp.wait()

    def cp_w(j, slot):
        return [
            pltpu.make_async_copy(src.bitcast(u32).at[:, j, :], w32.at[slot, pl.ds(r0, n)], sem_w.at[slot])
            for src, r0, n in ((wq_hbm, 0, M), (wk_hbm, M, DC), (wv_hbm, M + DC, DC))
        ]

    def wait_w(slot):
        pltpu.make_async_copy(w32.at[slot], w32.at[slot], sem_w.at[slot]).wait()

    def cp_oa(r0):
        return pltpu.make_async_copy(oa_s.at[pl.ds(r0, RST)], out_hbm.at[pl.ds(r0, RST), pl.ds(0, M)],
                                     sem_out.at[0])

    def cp_ob(c):
        return pltpu.make_async_copy(ob_s.at[pl.ds(c * PC, PC)], out_hbm.at[pl.ds(c * PC, PC), pl.ds(M, M)],
                                     sem_out.at[1])

    def unpack(r0, n, par, slot):
        w = w32[slot, r0:r0 + n, :]
        w = (w & jnp.uint32(HI_MASK)) if par else (w << 16)
        return pltpu.bitcast(w, f32)

    def ext_q(par, slot):
        wqh[par] = _pk(unpack(0, M, par, slot).astype(bf16))

    def ext_k(par, slot):
        wkh[par] = _pk(unpack(M, DC, par, slot).astype(bf16))

    def ext_v(par, slot):
        w = unpack(M + DC, DC, par, slot)
        for g in range(GC):
            wvth[par * GC + g] = _pk(w[g * 128:(g + 1) * 128, :].T.astype(bf16))

    def prep_t(sec):
        for cb in range(G):
            c0 = sec * M + cb * 128
            for g in range(G):
                t_s[g, c0:c0 + 128, :] = aw_s[g * 128:(g + 1) * 128, c0:c0 + 128].astype(f32).T

    def prep_g(sec):
        for d in range(DA):
            for g in range(G):
                wt_s[g, _half(sec * M + d * HA, HA), :] = _pk(
                    t_s[g, pl.ds(sec * M + d, HA, stride=DA), :].astype(bf16))

    def prep_w(sec):
        prep_t(sec)
        prep_g(sec)

    def prep_wo():
        for e in range(DA // 2):
            for g in range(G):
                w = awo_s[g, pl.ds(e, HA, stride=DA // 2), :]
                lo = pltpu.bitcast(w << 16, f32)
                hi = pltpu.bitcast(w & jnp.uint32(HI_MASK), f32)
                wop_s[g, _half(2 * e * HA, 2 * HA), :] = _pk(jnp.concatenate([lo, hi], axis=0).astype(bf16))

    def a_proj(rbase, secs, fine=False):
        chunks = [(0, PC), (PC, PC // 2), (PC + PC // 2, PC // 2)] if fine else [(0, PC), (PC, PC)]
        for sec in secs:
            for off, nr in chunks:
                r0 = rbase + off
                for n in range(G):
                    n0 = sec * M + n * 128
                    t = _tree([_mm_nt(_up(ax_s[g, _half(r0, nr), :]), _up(wt_s[g, _half(n0, 128), :]))
                               for g in range(G)], jnp.add)
                    if sec == 0:
                        qa_s[n, pl.ds(r0, nr), :] = t * QSCALE_A
                    elif sec == 1:
                        ka_s[n, pl.ds(r0 + PAD, nr), :] = t
                    else:
                        va_s[n, pl.ds(r0 + PAD, nr), :] = t

    def a_attn(rbase, never):
        outs = []
        prev = None
        for sub in range(RS // AG):
            rr = rbase + sub * AG
            q = [qa_s[g, pl.ds(rr, AG), :] for g in range(G)]
            if prev is not None:
                q = [jnp.where(never, prev, q[g]) for g in range(G)]
            lg = []
            for w in range(WIN):
                acc = _tree([q[g] * ka_s[g, pl.ds(rr + (PAD - DIL * w), AG), :] for g in range(G)], jnp.add)
                acc = acc + pltpu.roll(acc, 64, 1)
                acc = acc + pltpu.roll(acc, 32, 1)
                if w > 0 and sub * AG < PAD:
                    rowid = rr + lax.broadcasted_iota(jnp.int32, (AG, 128), 0)
                    acc = jnp.where(rowid >= DIL * w, acc, NEG)
                lg.append(acc)
            m = _tree(lg, jnp.maximum)
            e = [jnp.exp2(x - m) for x in lg]
            inv = pl.reciprocal(_tree(e, jnp.add), approx=False)
            og = []
            for g in range(G):
                acc = _tree([e[w] * va_s[g, pl.ds(rr + (PAD - DIL * w), AG), :] for w in range(WIN)], jnp.add)
                og.append(acc * inv)
            prev = og[-1]
            outs.append(jnp.concatenate(og, axis=1))
        return jnp.concatenate(outs, axis=0).astype(bf16)

    @pl.when(step == 0)
    def _prologue():
        start(cp_aw(0))
        start(cp_ax(0))
        z_s[0] = 0
        z_s[1] = 0
        zero = jnp.zeros((PAD, 128), f32)
        for g in range(G):
            ka_s[g, 0:PAD, :] = zero
            va_s[g, 0:PAD, :] = zero
        acc_ref[...] = jnp.zeros_like(acc_ref)
        wait(cp_aw(0))
        start(cp_aw(1))
        start(cp_ax(1))
        start(cp_aw(2))
        for c in range(2, NA):
            start(cp_ax(c))
        start(cp_awo)
        prep_w(0)
        wait(cp_ax(0))
        a_proj(0, (0,), fine=True)
        wait(cp_aw(1))
        wait(cp_ax(1))
        start(cp_w(0, 0))
        start(cp_b)
        a_proj(RA, (0,))
        prep_w(1)
        a_proj(0, (1,))
        wait(cp_aw(2))
        wait(cp_ax(2))
        wait(cp_awo)
        wait(cp_ax(3))
        a_proj(2 * RA, (0,))
        prep_wo()
        a_proj(3 * RA, (0,))
        prep_w(2)
        a_proj(0, (2,), fine=True)

        def body(c, carry):
            a_proj(pl.multiple_of(c * RA, RA), (1, 2))
            return carry
        lax.fori_loop(1, NA, body, 0)
        wait(cp_b)

    slot = step & 1
    wait_w(slot)

    @pl.when(step >= 1)
    def _():
        cp_oa(pl.multiple_of((step - 1) * RST, RST)).wait()

    def prefetch_w():
        @pl.when(step + 1 < NSTEP)
        def _():
            start(cp_w(step + 1, 1 - slot))

    zs = z_s[0]
    zl = z_s[1]
    never = zs != 0
    row = lax.broadcasted_iota(jnp.int32, (128, 128), 0)
    col = lax.broadcasted_iota(jnp.int32, (128, 128), 1)
    tri = row <= col

    obs = [{} for _ in range(HPS)]
    tokens = []
    clock = [0]

    def pub(r):
        tokens.append((clock[0], r[0:1, 0:128]))

    def token(lag):
        cand = [t for c0, t in tokens if c0 <= clock[0] - lag]
        return cand[-1] if cand else None

    def head(hh):
        h = step * HPS + hh
        sb = sbufs[4 * hh:4 * hh + 4]
        ra = pl.multiple_of(h * RS, RS)
        pm = {}
        mx = {}
        ot = {}
        ls = {}
        ob = obs[hh]
        oa = {}

        def Pq(a):
            def f():
                r = _tree([_mm(_up(bx_s[g, _half(a, PC), :]), _up(wqh[hh, _half(g * 128, 128), :]))
                           for g in range(G)], jnp.add)
                q_s[hh, _half(a, PC), :] = _pk((r * QSCALE_B).astype(bf16))
                pub(r)
            return (PC // 16 * G, f)

        def Pk(a):
            def f():
                r = _tree([_mm(_up(bc_s[g, _half(a, PC), :]), _up(wkh[hh, _half(g * 128, 128), :]))
                           for g in range(GC)], jnp.add)
                k_s[hh, _half(a, PC), :] = _pk(r.astype(bf16))
                pub(r)
            return (PC // 16 * GC, f)

        def Pv(a):
            def f():
                for j in range(a // 128, (a + PC) // 128):
                    r = _tree([_mm_nt(_up(wvth[hh * GC + g]), _up(bc_s[g, _half(j * 128, 128), :]))
                               for g in range(GC)], jnp.add)
                    vt_s[hh * 16 + j] = _pk(r.astype(bf16))
                pub(r)
            return (PC // 16 * GC, f)

        def QKq(i, k0, k1, t0):
            lo = i * BQ

            def f():
                r = _mm_nt(_up(k_s[hh, _half(k0, k1 - k0), :]),
                           _up(q_s[hh, _half(lo + t0 * 128, BQ - t0 * 128), :]))
                pub(r)
                for t in range(t0, 4):
                    c = i * 4 + t
                    for j in range(k0 // 128, k1 // 128):
                        tile = r[j * 128 - k0:(j + 1) * 128 - k0, (t - t0) * 128:(t - t0 + 1) * 128]
                        if j == c:
                            tile = jnp.where(tri, tile, NEG)
                        sb[i][zs + t, j * 128:(j + 1) * 128, :] = tile
                        pm.setdefault(c, []).append(_fold8(tile, jnp.maximum))
            return ((k1 - k0) // 16 * (4 - t0), f)

        def QK(i):
            lo = i * BQ
            qs = []
            k0 = 0
            while k0 < lo + 128:
                k1 = min(k0 + KC, lo + 128)
                qs.append(QKq(i, k0, k1, 0))
                k0 = k1
            for u in range(1, 4):
                qs.append(QKq(i, lo + u * 128, lo + (u + 1) * 128, u))
            return qs

        def PVq(c, j0, j1):
            def f():
                if c not in mx:
                    mx[c] = jnp.max(_tree(pm.pop(c), jnp.maximum), axis=0, keepdims=True)
                m = mx[c]
                tok = token(LAGC)
                if tok is not None:
                    m = jnp.where(never, tok, m)
                ps = [jnp.exp2(sb[c // 4][zl + c % 4, j * 128:(j + 1) * 128, :] - m) for j in range(j0, j1)]
                lsum = _tree([_fold8(p, jnp.add) for p in ps], jnp.add)
                ls[c] = lsum if c not in ls else ls[c] + lsum
                o = _tree([_mm(_up(vt_s[hh * 16 + j]), p.astype(bf16)) for j, p in zip(range(j0, j1), ps)],
                          jnp.add)
                pub(o)
                ot[c] = o if c not in ot else ot[c] + o
                if j1 == c + 1:
                    l = jnp.sum(ls.pop(c), axis=0, keepdims=True)
                    ob[c] = (ot.pop(c) * pl.reciprocal(l, approx=False)).T
            return ((j1 - j0) * 8, f)

        def PV(i):
            qs = []
            for t in range(4):
                c = i * 4 + t
                for j0 in range(0, c + 1, PVK):
                    qs.append(PVq(c, j0, min(j0 + PVK, c + 1)))
            return qs

        def OPq(a):
            def f():
                cs = range(a // 128, (a + PC) // 128)
                os_ = [jnp.concatenate([obs[u].pop(c) for c in cs], axis=0).astype(bf16) for u in range(HPS)]
                for g in range(G):
                    new = acc_ref[a:a + PC, g * 128:(g + 1) * 128] + _tree(
                        [_mm(os_[u], _up(wo_s[g, step * HPS + u])) for u in range(HPS)], jnp.add)
                    acc_ref[a:a + PC, g * 128:(g + 1) * 128] = new
                    if g == 0:
                        pub(new)
                    ob_s[a:a + PC, g * 128:(g + 1) * 128] = new.astype(bf16)

                @pl.when(step == NSTEP - 1)
                def _():
                    cp_ob(a // PC).start()
            return (PC // 16 * G * HPS, f)

        def do(fn, *args):
            return (0, lambda: fn(*args))

        def Aattn():
            oa[0] = a_attn(ra, never)

        def Aout():
            o = oa.pop(0)
            for g in range(G):
                oa_s[pl.ds(ra, RS), g * 128:(g + 1) * 128] = _mm(o, _up(wop_s[g])).astype(bf16)
            if hh == HPS - 1:
                cp_oa(pl.multiple_of(step * RST, RST)).start()

        def rows(i):
            return range(i * BQ, (i + 1) * BQ, PC)

        return dict(
            ext=[do(ext_q, hh, slot), do(ext_k, hh, slot), do(ext_v, hh, slot), do(Aattn)],
            aout=[do(Aout)],
            pq=lambda i: [Pq(a) for a in rows(i)],
            op=lambda i: [OPq(a) for a in rows(i)],
            QK=QK, PV=PV,
            pk=[Pk(a) for a in range(0, S, PC)],
            pv=[Pv(a) for a in range(0, S, PC)])

    A = head(0)
    B = head(1)
    pre_a = A['pq'](3) + A['pk'] + A['aout'] + A['QK'](3) + A['pq'](2) + A['pv']
    pre_b = [(0, prefetch_w)] + B['ext'] + B['pq'](3) + B['pk'] + B['aout'] + B['QK'](3) + B['pq'](2) + B['pv']
    seq = A['ext'] + pre_a
    seq += _interleave(A['PV'](3), A['pq'](1) + A['QK'](2))
    seq += _interleave(A['PV'](2), A['pq'](0) + A['QK'](1) + pre_b[:6])
    seq += _interleave(A['PV'](1), A['QK'](0) + pre_b[6:9])
    seq += _interleave(A['PV'](0), pre_b[9:12])
    seq += pre_b[12:]
    seq += _interleave(B['PV'](3), B['QK'](2) + B['pq'](1))
    seq += _interleave(B['PV'](2), B['pq'](0) + B['QK'](1) + B['op'](3))
    seq += _interleave(B['PV'](1), B['QK'](0) + B['op'](2))
    seq += B['PV'](0) + B['op'](1) + B['op'](0)
    for cost, f in seq:
        f()
        clock[0] += cost

    @pl.when(step == NSTEP - 1)
    def _epilogue():
        cp_oa((NSTEP - 1) * RST).wait()
        pltpu.make_async_copy(ob_s, out_hbm.at[:, pl.ds(M, M)], sem_out.at[1]).wait()


@jax.jit
def pallas_concat_heads__sliding_local_dilated__compressed_kv_cla__prompt_kernel(
    A_x: jax.Array,
    A_wqkv: jax.Array,
    A_wo: jax.Array,
    B_x: jax.Array,
    B_c_kv: jax.Array,
    B_w_q: jax.Array,
    B_w_uk: jax.Array,
    B_w_uv: jax.Array,
    B_w_o: jax.Array,
):
    any_spec = pl.BlockSpec(memory_space=pl.ANY)
    scratch = [
        pltpu.VMEM((G, S // 2, 128), u32),
        pltpu.VMEM((M, 3 * M), bf16),
        pltpu.VMEM((G, M // 2 + 32, 128), u32),
        pltpu.VMEM((G, 3 * M + 32, 128), f32),
        pltpu.VMEM((G, 3 * M // 2, 128), u32),
        pltpu.VMEM((G, M // 2, 128), u32),
        pltpu.VMEM((G, S, 128), f32),
        pltpu.VMEM((G, S + 2 * PAD, 128), f32),
        pltpu.VMEM((G, S + 2 * PAD, 128), f32),
        pltpu.VMEM((S, M), bf16),
        pltpu.VMEM((G, S // 2, 128), u32),
        pltpu.VMEM((GC, S // 2, 128), u32),
        pltpu.VMEM((2, M + 2 * DC, D), u32),
        pltpu.VMEM((G, H, D // 2, 128), u32),
        pltpu.VMEM((HPS, M // 2, D), u32),
        pltpu.VMEM((HPS, DC // 2, D), u32),
        pltpu.VMEM((HPS * GC, D // 2, 128), u32),
        pltpu.VMEM((HPS, S // 2, D), u32),
        pltpu.VMEM((HPS, S // 2, D), u32),
        pltpu.VMEM((HPS * S // 128, D // 2, 128), u32),
        pltpu.VMEM((S, M), f32),
        pltpu.VMEM((S, M), bf16),
        pltpu.SMEM((2,), jnp.int32),
        pltpu.SemaphoreType.DMA((5 + NA,)),
        pltpu.SemaphoreType.DMA((2,)),
        pltpu.SemaphoreType.DMA((2,)),
    ]
    scratch += [pltpu.VMEM((4, (i + 1) * BQ, 128), f32) for _ in range(HPS) for i in range(4)]
    out = pl.pallas_call(
        _kernel,
        grid=(NSTEP,),
        in_specs=[any_spec] * 9,
        out_specs=any_spec,
        out_shape=jax.ShapeDtypeStruct((S, 2 * M), bf16),
        scratch_shapes=scratch,
        compiler_params=pltpu.CompilerParams(
            dimension_semantics=("arbitrary",), vmem_limit_bytes=110 * 1024 * 1024),
    )(A_x.reshape(S, M), A_wqkv, A_wo, B_x.reshape(S, M), B_c_kv.reshape(S, DC),
      B_w_q, B_w_uk, B_w_uv, B_w_o)
    return out.reshape(1, S, 2 * M)
```
